```python
import os as _os
_os.environ.setdefault("JAX_PLATFORMS", "cpu")
import jax
import jax.numpy as jnp

def _softmax(x, axis=-1):
    return jax.nn.softmax(x, axis=axis)
def _gelu(x):
    return jax.nn.gelu(x, approximate=True)
def _silu(x):
    return jax.nn.silu(x)
def _sigmoid(x):
    return jax.nn.sigmoid(x)
def _layernorm(x, axis=-1, eps=1e-5):
    m = jnp.mean(x, axis=axis, keepdims=True)
    v = jnp.var(x, axis=axis, keepdims=True)
    return (x - m) / jnp.sqrt(v + eps)
def _scatter_add(tgt, idx, src, axis=0):
    return tgt.at[idx].add(src)
def _segment_sum(src, seg, n):
    return jax.ops.segment_sum(src, seg, n)
class _Rng:
    def __init__(self, key):
        self._k = key
    def _next(self):
        self._k, sub = jax.random.split(self._k)
        return sub
    def normal(self, shape):
        return jax.random.normal(self._next(), shape, dtype=jnp.bfloat16)
    def randint(self, lo, hi, shape):
        return jax.random.randint(self._next(), shape, lo, hi, dtype=jnp.int32)
    def uniform(self, shape, lo=0.0, hi=1.0):
        return jax.random.uniform(self._next(), shape, jnp.bfloat16, lo, hi)
    def permutation(self, n):
        return jax.random.permutation(self._next(), n)


kernel_name = 'standalone__gqa_softmax__near_ridge'

def setup_inputs():
    _rng = _Rng(jax.random.key(int.from_bytes(__import__("os").urandom(4), "little")))
    _w = (lambda a: (lambda t: t.astype(jnp.bfloat16) if jnp.issubdtype(t.dtype, jnp.floating) else t)(jnp.asarray(a)))
    B, Hq, Hkv, Sq, Sk, D = 8, 32, 8, 112, 2048, 128
    return {
        "q": _w((lambda *s: _rng.normal(s) * 0.4)(B, Hq, Sq, D)),
        "k": _w((lambda *s: _rng.normal(s) * 0.4)(B, Hkv, Sk, D)),
        "v": _w((lambda *s: _rng.normal(s) * 0.05)(B, Hkv, Sk, D)),
    }

def reference(q, k, v):
    B, Hq, Sq, D = q.shape
    Hkv = k.shape[1]
    rep = Hq // Hkv
    k = jnp.repeat(k, rep, axis=1)
    v = jnp.repeat(v, rep, axis=1)
    scale = D ** -0.5
    scores = jnp.einsum("bhqd,bhkd->bhqk", q, k) * scale
    p = _softmax(scores, axis=-1)
    return jnp.einsum("bhqk,bhkd->bhqd", p, v)
```

```python
import functools
import jax, jax.numpy as jnp
from jax import lax
from jax.experimental import pallas as pl
from jax.experimental.pallas import tpu as pltpu
LOG2E = 1.4426950408889634
NT = (((1,), (1,)), ((), ()))
F32 = jnp.float32

def make(kc=512, order="qsp", vmem=100, U=2, fin_pos="start", midwait=False, flags=None, nr=True, mfin_pos='start'):
    NS = 2
    def kern(q_hbm, k_hbm, v_hbm, o_hbm, qb, kb, vb, ob, sA, sB, mA, mB, lA, lB, oA, oB, sq, sk, sv, so, *, c, G):
        R, D = qb.shape[2], qb.shape[3]
        Sk = kb.shape[2]
        T = Sk // kc
        def tile_reduce(x, op):
            r = x[:, 0:128]
            for i in range(1, x.shape[1] // 128):
                r = op(r, x[:, i*128:(i+1)*128])
            return r
        def qk_t(t, q_ref, k_ref, s_w, m_w):
            q = q_ref[...]
            k = k_ref[t*kc:(t+1)*kc, :]
            s = lax.dot_general(q, k, NT, preferred_element_type=F32)
            s_w[:, t*kc:(t+1)*kc] = s
            mx = tile_reduce(s, jnp.maximum)
            if t > 0:
                mx = jnp.maximum(mx, m_w[...])
            if mfin_pos == 'end' and t == T - 1:
                mx = jnp.broadcast_to(jnp.max(mx, axis=-1, keepdims=True), mx.shape)
            m_w[...] = mx
        def m_fin(m_r):
            m_r[...] = jnp.broadcast_to(jnp.max(m_r[...], axis=-1, keepdims=True), m_r.shape)
        def sm_t(t, s_r, m_r, lacc):
            s = s_r[:, t*kc:(t+1)*kc]
            m = m_r[...]
            m = jnp.concatenate([m] * (kc // 128), axis=1)
            p = jnp.exp2((s - m) * c)
            ls = tile_reduce(p, jnp.add)
            if t > 0:
                ls = ls + lacc[...]
            lacc[...] = ls
            return p.astype(jnp.bfloat16)
        def pv_t(t, v_ref, p, oacc):
            v = v_ref[t*kc:(t+1)*kc, :]
            o = jnp.dot(p, v, preferred_element_type=F32)
            if t > 0:
                o = o + oacc[...]
            oacc[...] = o
        def fin(lacc, oacc, dst):
            l = jnp.sum(lacc[...], axis=-1, keepdims=True)
            if nr:
                r = pl.reciprocal(l, approx=True)
                r = r * (2.0 - l * r)
                dst[...] = (oacc[...] * r).astype(dst.dtype)
            else:
                dst[...] = (oacc[...] / l).astype(dst.dtype)
        SB = [(sA, mA, lA, oA), (sB, mB, lB, oB)]
        def phase(par, q_ref, k_ref, v_ref, dst, do_qk=True, do_pv=True, do_fin=True):
            s_w, m_w, l_f, o_f = SB[par]
            s_r, m_r, l_a, o_a = SB[1 - par]
            if do_pv and mfin_pos == 'start': m_fin(m_r)
            if do_fin and fin_pos == "start": fin(l_f, o_f, dst)
            for t in range(T):
                for ch in order:
                    if ch == "q" and do_qk: qk_t(t, q_ref, k_ref, s_w, m_w)
                    if ch == "s" and do_pv: p = sm_t(t, s_r, m_r, l_a)
                    if ch == "p" and do_pv: pv_t(t, v_ref, p, o_a)
                if do_fin and fin_pos == "mid" and t == 0: fin(l_f, o_f, dst)
        def in_copies(j, slot):
            return (pltpu.make_async_copy(q_hbm.at[pl.ds(j*U, U)], qb.at[slot], sq.at[slot]),
                    pltpu.make_async_copy(k_hbm.at[pl.ds(j*U, U)], kb.at[slot], sk.at[slot]),
                    pltpu.make_async_copy(v_hbm.at[pl.ds(j*U, U)], vb.at[slot], sv.at[slot]))
        def out_copy(j, slot):
            return pltpu.make_async_copy(ob.at[slot], o_hbm.at[pl.ds(j*U, U)], so.at[slot])
        NJ = G // U
        def iteration(j, slot, pslot, first=False, last=False):
            for u in range(U):
                n_par = u % 2
                q_ref = qb.at[slot, u]; k_ref = kb.at[slot, u]
                v_ref = vb.at[pslot, U - 1] if u == 0 else vb.at[slot, u - 1]
                if u < 2: dst = ob.at[pslot, (u - 2) % U]
                else: dst = ob.at[slot, u - 2]
                phase(n_par, q_ref, k_ref, v_ref, dst, do_qk=True, do_pv=not (first and u == 0), do_fin=not (first and u < 2))
                if u == 1 and not first:
                    out_copy(j - 1, pslot).start()
        for cpy in in_copies(0, 0): cpy.start()
        for cpy in in_copies(1, 1): cpy.start()
        for cpy in in_copies(0, 0): cpy.wait()
        iteration(0, 0, 1, first=True)
        def loop_body(j, carry):
            slot = lax.rem(j, 3); pslot = lax.rem(j + 2, 3); nslot = lax.rem(j + 1, 3)
            for cpy in in_copies(j, slot): cpy.wait()
            @pl.when(j + 1 < NJ)
            def _():
                for cpy in in_copies(j + 1, nslot): cpy.start()
            @pl.when(j >= 3)
            def _(): out_copy(j - 3, slot).wait()
            iteration(j, slot, pslot)
            return carry
        lax.fori_loop(1, NJ, loop_body, None)
        ls = (NJ - 1) % 3
        phase(0, None, None, vb.at[ls, U - 1], ob.at[ls, U - 2], do_qk=False)
        fin(lB, oB, ob.at[ls, U - 1])
        out_copy(NJ - 1, ls).start()
        out_copy(NJ - 3, (NJ - 3) % 3).wait()
        out_copy(NJ - 2, (NJ - 2) % 3).wait()
        out_copy(NJ - 1, ls).wait()

    def fn(q, k, v):
        B, Hq, Sq, D = q.shape
        Hkv, Sk = k.shape[1], k.shape[2]
        G = B * Hkv; R = (Hq // Hkv) * Sq
        c = float(D ** -0.5) * LOG2E
        out = pl.pallas_call(
            functools.partial(kern, c=c, G=G),
            in_specs=[pl.BlockSpec(memory_space=pl.ANY)] * 3,
            out_specs=pl.BlockSpec(memory_space=pl.ANY),
            out_shape=jax.ShapeDtypeStruct((G, R, D), q.dtype),
            scratch_shapes=[
                pltpu.VMEM((3, U, R, D), jnp.bfloat16), pltpu.VMEM((3, U, Sk, D), jnp.bfloat16), pltpu.VMEM((3, U, Sk, D), jnp.bfloat16),
                pltpu.VMEM((3, U, R, D), jnp.bfloat16),
                pltpu.VMEM((R, Sk), F32), pltpu.VMEM((R, Sk), F32),
                pltpu.VMEM((R, 128), F32), pltpu.VMEM((R, 128), F32),
                pltpu.VMEM((R, 128), F32), pltpu.VMEM((R, 128), F32),
                pltpu.VMEM((R, 128), F32), pltpu.VMEM((R, 128), F32),
                pltpu.SemaphoreType.DMA((3,)), pltpu.SemaphoreType.DMA((3,)), pltpu.SemaphoreType.DMA((3,)), pltpu.SemaphoreType.DMA((3,)),
            ],
            compiler_params=pltpu.CompilerParams(vmem_limit_bytes=vmem*2**20, flags=flags),
        )(q.reshape(G, R, D), k.reshape(G, Sk, D), v.reshape(G, Sk, D))
        return out.reshape(B, Hq, Sq, D)
    return fn


_impl = make(512, "qsp", fin_pos="mid", flags={"XLA_TPU_FORCE_LP_LLO_SCHEDULER": True}, mfin_pos="end")


@jax.jit
def pallas_standalone__gqa_softmax__near_ridge_kernel(q, k, v):
    return _impl(q, k, v)
```

```python
import functools

import jax
import jax.numpy as jnp
from jax import lax
from jax.experimental import pallas as pl
from jax.experimental.pallas import tpu as pltpu

LOG2E = 1.4426950408889634
NT = (((1,), (1,)), ((), ()))
F32 = jnp.float32
BF16 = jnp.bfloat16
KC = 512
U = 2
LANES = 128


def _tile_reduce(x, op):
    r = x[:, 0:LANES]
    for i in range(1, x.shape[1] // LANES):
        r = op(r, x[:, i * LANES:(i + 1) * LANES])
    return r


def _zero_bits(v):
    b = pltpu.bitcast(v, jnp.uint32)
    return lax.shift_right_logical(lax.shift_right_logical(b, jnp.uint32(31)), jnp.uint32(1))


def _kernel(q_hbm, k_hbm, v_hbm, o_hbm, qb, kb, vb, ob,
            sA, mA, lA, oA, sB, mB, lB, oB, sq, sk, sv, so, s0, *, c, G):
    Sk = kb.shape[2]
    T = Sk // KC
    NJ = G // U
    sets = [(sA, mA, lA, oA), (sB, mB, lB, oB)]

    def qk_t(t, q_ref, k_ref, s_w, m_w):
        s = lax.dot_general(q_ref[...], k_ref[t * KC:(t + 1) * KC, :], NT,
                            preferred_element_type=F32)
        s_w[:, t * KC:(t + 1) * KC] = s
        mx = _tile_reduce(s, jnp.maximum)
        if t > 0:
            mx = jnp.maximum(mx, m_w[...])
        if t == T - 1:
            mx = jnp.broadcast_to(jnp.max(mx, axis=-1, keepdims=True), mx.shape)
        m_w[...] = mx
        return mx

    def sm_t(t, s_r, m_r, lacc, dep):
        s = s_r[:, t * KC:(t + 1) * KC]
        m = m_r[...]
        if dep is not None:
            m = pltpu.bitcast(pltpu.bitcast(m, jnp.uint32) | _zero_bits(dep), F32)
        m = jnp.concatenate([m] * (KC // LANES), axis=1)
        p = jnp.exp2((s - m) * c)
        ls = _tile_reduce(p, jnp.add)
        if t > 0:
            ls = ls + lacc[...]
        lacc[...] = ls
        return p.astype(BF16)

    def pv_t(t, v_ref, p, oacc):
        o = jnp.dot(p, v_ref[t * KC:(t + 1) * KC, :], preferred_element_type=F32)
        if t > 0:
            o = o + oacc[...]
        oacc[...] = o

    def fin(lacc, oacc, dst):
        l = jnp.sum(lacc[...], axis=-1, keepdims=True)
        r = pl.reciprocal(l, approx=True)
        r = r * (2.0 - l * r)
        dst[...] = (oacc[...] * r).astype(dst.dtype)

    def phase(par, q_ref, k_ref, v_ref, dst, do_qk=True, do_pv=True, do_fin=True, hook=None):
        s_w, m_w, l_f, o_f = sets[par]
        s_r, m_r, l_a, o_a = sets[1 - par]
        for t in range(T):
            if hook is not None:
                hook(t)
            mx = qk_t(t, q_ref, k_ref, s_w, m_w) if do_qk else None
            if do_fin and t == 0:
                fin(l_f, o_f, dst)
            if do_pv:
                p = sm_t(t, s_r, m_r, l_a, mx if t == 0 else None)
                pv_t(t, v_ref, p, o_a)

    def in_copies(j, slot):
        return (pltpu.make_async_copy(q_hbm.at[pl.ds(j * U, U)], qb.at[slot], sq.at[slot]),
                pltpu.make_async_copy(k_hbm.at[pl.ds(j * U, U)], kb.at[slot], sk.at[slot]),
                pltpu.make_async_copy(v_hbm.at[pl.ds(j * U - 1, U)], vb.at[slot], sv.at[slot]))

    def out_copy(j, slot):
        return pltpu.make_async_copy(ob.at[slot], o_hbm.at[pl.ds(j * U, U)], so.at[slot])

    small = []

    def fetch(src, dst):
        cp = pltpu.make_async_copy(src, dst, s0.at[len(small)])
        small.append(cp)
        cp.start()
        return cp

    cq0 = fetch(q_hbm.at[0], qb.at[0, 0])
    ck0 = [fetch(k_hbm.at[0, t * KC:(t + 1) * KC], kb.at[0, 0, t * KC:(t + 1) * KC])
           for t in range(T)]
    late = []

    def hook0(t):
        if t == 0:
            cq0.wait()
        ck0[t].wait()
        if t == 0:
            late.append(fetch(q_hbm.at[1], qb.at[0, 1]))
            late.append(fetch(k_hbm.at[1], kb.at[0, 1]))
            late.append(fetch(v_hbm.at[0], vb.at[0, 1]))

    phase(0, qb.at[0, 0], kb.at[0, 0], None, None, do_pv=False, do_fin=False, hook=hook0)
    for cp in late:
        cp.wait()
    for cp in in_copies(1, 1):
        cp.start()
    phase(1, qb.at[0, 1], kb.at[0, 1], vb.at[0, 1], None, do_fin=False)
    for cp in in_copies(2, 2):
        cp.start()

    def v_last(slot):
        return pltpu.make_async_copy(v_hbm.at[G - 1], vb.at[slot, 0], sv.at[slot])

    def loop_body(j, carry):
        pslot, slot, nslot = carry
        for cp in in_copies(j, slot):
            cp.wait()

        @pl.when(j >= 3)
        def _():
            out_copy(j - 3, slot).wait()

        for u in range(U):
            phase(u, qb.at[slot, u], kb.at[slot, u], vb.at[slot, u], ob.at[pslot, u])
        out_copy(j - 1, pslot).start()

        @pl.when(j + 2 < NJ)
        def _():
            for cp in in_copies(j + 2, pslot):
                cp.start()

        @pl.when(j + 2 == NJ)
        def _():
            v_last(pslot).start()

        return (slot, nslot, pslot)

    lax.fori_loop(1, NJ, loop_body, (0, 1, 2))

    ls_, es = (NJ - 1) % 3, NJ % 3
    v_last(es).wait()
    phase(0, None, None, vb.at[es, 0], ob.at[ls_, 0], do_qk=False)
    e0 = pltpu.make_async_copy(ob.at[ls_, 0], o_hbm.at[G - 2], s0.at[0])
    e0.start()
    fin(lB, oB, ob.at[ls_, 1])
    e1 = pltpu.make_async_copy(ob.at[ls_, 1], o_hbm.at[G - 1], s0.at[1])
    e1.start()
    out_copy(NJ - 3, (NJ - 3) % 3).wait()
    out_copy(NJ - 2, (NJ - 2) % 3).wait()
    e0.wait()
    e1.wait()


@jax.jit
def pallas_standalone__gqa_softmax__near_ridge_kernel(q, k, v):
    B, Hq, Sq, D = q.shape
    Hkv, Sk = k.shape[1], k.shape[2]
    G, R = B * Hkv, (Hq // Hkv) * Sq
    T = Sk // KC
    c = float(D ** -0.5) * LOG2E
    one_set = [pltpu.VMEM((R, Sk), F32), pltpu.VMEM((R, LANES), F32),
               pltpu.VMEM((R, LANES), F32), pltpu.VMEM((R, D), F32)]
    out = pl.pallas_call(
        functools.partial(_kernel, c=c, G=G),
        in_specs=[pl.BlockSpec(memory_space=pl.ANY)] * 3,
        out_specs=pl.BlockSpec(memory_space=pl.ANY),
        out_shape=jax.ShapeDtypeStruct((G, R, D), q.dtype),
        scratch_shapes=[
            pltpu.VMEM((3, U, R, D), BF16), pltpu.VMEM((3, U, Sk, D), BF16),
            pltpu.VMEM((3, U, Sk, D), BF16), pltpu.VMEM((3, U, R, D), BF16),
            *one_set, *one_set,
            pltpu.SemaphoreType.DMA((3,)), pltpu.SemaphoreType.DMA((3,)),
            pltpu.SemaphoreType.DMA((3,)), pltpu.SemaphoreType.DMA((3,)),
            pltpu.SemaphoreType.DMA((T + 4,)),
        ],
        compiler_params=pltpu.CompilerParams(
            vmem_limit_bytes=100 * 2**20,
            disable_bounds_checks=True,
            flags={"XLA_TPU_FORCE_LP_LLO_SCHEDULER": True}),
    )(q.reshape(G, R, D), k.reshape(G, Sk, D), v.reshape(G, Sk, D))
    return out.reshape(B, Hq, Sq, D)
```
